```python
import os as _os
_os.environ.setdefault("JAX_PLATFORMS", "cpu")
import jax
import jax.numpy as jnp

def _softmax(x, axis=-1):
    return jax.nn.softmax(x, axis=axis)
def _gelu(x):
    return jax.nn.gelu(x, approximate=True)
def _silu(x):
    return jax.nn.silu(x)
def _sigmoid(x):
    return jax.nn.sigmoid(x)
def _layernorm(x, axis=-1, eps=1e-5):
    m = jnp.mean(x, axis=axis, keepdims=True)
    v = jnp.var(x, axis=axis, keepdims=True)
    return (x - m) / jnp.sqrt(v + eps)
def _scatter_add(tgt, idx, src, axis=0):
    return tgt.at[idx].add(src)
def _segment_sum(src, seg, n):
    return jax.ops.segment_sum(src, seg, n)
class _Rng:
    def __init__(self, key):
        self._k = key
    def _next(self):
        self._k, sub = jax.random.split(self._k)
        return sub
    def normal(self, shape):
        return jax.random.normal(self._next(), shape, dtype=jnp.bfloat16)
    def randint(self, lo, hi, shape):
        return jax.random.randint(self._next(), shape, lo, hi, dtype=jnp.int32)
    def uniform(self, shape, lo=0.0, hi=1.0):
        return jax.random.uniform(self._next(), shape, jnp.bfloat16, lo, hi)
    def permutation(self, n):
        return jax.random.permutation(self._next(), n)


kernel_name = 'concat_heads__mha_block_cached__mha_block_cached__near_ridge'

def setup_inputs():
    _rng = _Rng(jax.random.key(int.from_bytes(__import__("os").urandom(4), "little")))
    _w = (lambda a: (lambda t: t.astype(jnp.bfloat16) if jnp.issubdtype(t.dtype, jnp.floating) else t)(jnp.asarray(a)))
    def _A_setup():
        B, Sq, D = 32, 32, 640
        H, Sk, Dh = 32, 32, 128
        return {
            "x": _w((lambda *s: _rng.normal(s) * 0.8)(B, Sq, D)),
            "k_cache": _w((lambda *s: _rng.normal(s) * 0.8)(B, H, Sk, Dh)),
            "v_cache": _w((lambda *s: _rng.normal(s) * 0.05)(B, H, Sk, Dh)),
            "wq": _w((lambda *s: _rng.normal(s) * 0.8)(D, H * Dh) * (D ** -0.5)),
            "wo": _w((lambda *s: _rng.normal(s) * 0.05)(H * Dh, D) * ((H * Dh) ** -0.5)),
        }
    _A_in = _A_setup()

    def _B_setup():
        B, Sq, D = 32, 32, 640
        H, Sk, Dh = 32, 32, 128
        return {
            "x": _w((lambda *s: _rng.normal(s) * 0.8)(B, Sq, D)),
            "k_cache": _w((lambda *s: _rng.normal(s) * 0.8)(B, H, Sk, Dh)),
            "v_cache": _w((lambda *s: _rng.normal(s) * 0.05)(B, H, Sk, Dh)),
            "wq": _w((lambda *s: _rng.normal(s) * 0.8)(D, H * Dh) * (D ** -0.5)),
            "wo": _w((lambda *s: _rng.normal(s) * 0.05)(H * Dh, D) * ((H * Dh) ** -0.5)),
        }
    _B_in = _B_setup()

    return {
        "A_x": _A_in["x"],
        "A_k_cache": _A_in["k_cache"],
        "A_v_cache": _A_in["v_cache"],
        "A_wq": _A_in["wq"],
        "A_wo": _A_in["wo"],
        "B_x": _B_in["x"],
        "B_k_cache": _B_in["k_cache"],
        "B_v_cache": _B_in["v_cache"],
        "B_wq": _B_in["wq"],
        "B_wo": _B_in["wo"],
    }

def reference(A_x, A_k_cache, A_v_cache, A_wq, A_wo, B_x, B_k_cache, B_v_cache, B_wq, B_wo):
    def _A_ref(x, k_cache, v_cache, wq, wo):
        B, Sq, D = x.shape
        H, Dh = 32, 128
        q = (lambda x, *d: x.transpose(*d))((x @ wq).reshape(B, Sq, H, Dh), 0, 2, 1, 3)
        scores = jnp.einsum("bhqd,bhkd->bhqk", q, k_cache) * (Dh ** -0.5)
        p = _softmax(scores, axis=-1)
        o = jnp.einsum("bhqk,bhkd->bhqd", p, v_cache)
        return (lambda x, *d: x.transpose(*d))(o, 0, 2, 1, 3).reshape(B, Sq, H * Dh) @ wo

    def _B_ref(x, k_cache, v_cache, wq, wo):
        B, Sq, D = x.shape
        H, Dh = 32, 128
        q = (lambda x, *d: x.transpose(*d))((x @ wq).reshape(B, Sq, H, Dh), 0, 2, 1, 3)
        scores = jnp.einsum("bhqd,bhkd->bhqk", q, k_cache) * (Dh ** -0.5)
        p = _softmax(scores, axis=-1)
        o = jnp.einsum("bhqk,bhkd->bhqd", p, v_cache)
        return (lambda x, *d: x.transpose(*d))(o, 0, 2, 1, 3).reshape(B, Sq, H * Dh) @ wo

    a = _A_ref(A_x, A_k_cache, A_v_cache, A_wq, A_wo)
    b = _B_ref(B_x, B_k_cache, B_v_cache, B_wq, B_wo)
    return jnp.concatenate([a, b], axis=-1)
```

```python
import jax
import jax.numpy as jnp
import numpy as np
import jax.experimental.pallas as pl
import jax.experimental.pallas.tpu as pltpu

B, SQ, D, H, SK, DH = 32, 32, 640, 32, 32, 128
M = B * SQ
NQ = B // 4
LOG2E = 1.4426950408889634
f32, bf16, u32 = jnp.float32, jnp.bfloat16, jnp.uint32
C = DH ** -0.5 * LOG2E

def make(G=4, L=2, XC=4, OC=(512, 256, 128, 128), kv32=True, rcp_approx=False, LA=2, nobc=True, qT=False):
    NG = H // G
    NS = 2 * NG
    W = G * DH
    assert LA >= L
    def kern(xa, ka, va, wqa, woa, xb, kb, vb, wqb, wob, out,
             x_buf, k_buf, v_buf, wq_buf, wo_buf, q_buf, acc, o_buf, sems, xsem, osem):
        srcs = ((xa, ka, va, wqa, woa), (xb, kb, vb, wqb, wob))
        RX = M // XC
        def copy(s, i):
            _, ks, vs, wqs, wos = srcs[s // NG]
            g = s % NG
            if i == 0: return pltpu.make_async_copy(wqs.at[:, pl.ds(g * W, W)], wq_buf.at[s], sems.at[0, s])
            if i == 1: return pltpu.make_async_copy(ks.at[:, pl.ds(g * G, G)], k_buf.at[s], sems.at[1, s])
            if i == 2: return pltpu.make_async_copy(vs.at[:, pl.ds(g * G, G)], v_buf.at[s], sems.at[2, s])
            if i == 3: return pltpu.make_async_copy(wos.at[pl.ds(g * W, W), :], wo_buf.at[s], sems.at[3, s])
        def wait(s, i):
            dst = (wq_buf, k_buf, v_buf, wo_buf)[i].at[s]
            pltpu.make_async_copy(dst, dst, sems.at[i, s]).wait()
        xa_c = [pltpu.make_async_copy(xa.at[pl.ds(c * RX, RX)], x_buf.at[0, pl.ds(c * RX, RX)], sems.at[4, 1 + c]) for c in range(XC)]
        xb_c = pltpu.make_async_copy(xb, x_buf.at[1], sems.at[4, 0])

        lane = jax.lax.broadcasted_iota(jnp.int32, (32, 128), 1)
        msk = [lane // 32 == i for i in range(4)]
        def ldkv(buf, s, h, j):
            if kv32:
                return pltpu.bitcast(buf.bitcast(u32)[s, 4*j:4*j+4, h].reshape(64, 128), bf16)
            return buf[s, 4*j:4*j+4, h].reshape(128, 128)
        def qproj(s, slot, r0=0, nr=M):
            q = jnp.dot(x_buf[s // NG, r0:r0 + nr], wq_buf[s], preferred_element_type=f32)
            if not qT:
                q_buf[slot, r0:r0 + nr] = q.astype(bf16)
                return
            for h in range(G):
                for j in range(nr // 128):
                    t = q[j*128:(j+1)*128, h*128:(h+1)*128].astype(bf16).T
                    q_buf[slot, h, r0 // 128 + j] = pltpu.bitcast(t, u32)
        def soft(s, slot, h, j):
            kt = ldkv(k_buf, s, h, j)
            if qT:
                st = jnp.dot(kt, pltpu.bitcast(q_buf[slot, h, j], bf16), preferred_element_type=f32)
            else:
                qt = q_buf[slot, j*128:(j+1)*128, h*128:(h+1)*128]
                st = jax.lax.dot_general(kt, qt, (((1,), (1,)), ((), ())), preferred_element_type=f32)
            ct = jnp.where(msk[0], st[0:32], jnp.where(msk[1], st[32:64], jnp.where(msk[2], st[64:96], st[96:128])))
            m = jnp.max(ct, axis=0, keepdims=True)
            e = jnp.exp2((ct - m) * C)
            l = jnp.sum(e, axis=0, keepdims=True)
            return e * pl.reciprocal(l, approx=rcp_approx)
        def pv(s, h, j, pb):
            vt = ldkv(v_buf, s, h, j)
            ptb = jnp.concatenate([jnp.where(msk[i], pb, 0.0) for i in range(4)], axis=0).astype(bf16)
            return jax.lax.dot_general(ptb, vt, (((0,), (0,)), ((), ())), preferred_element_type=f32)
        def attn(s, slot):
            hj = [(h, j) for h in range(G) for j in range(NQ)]
            ps = {t: soft(s, slot, *t) for t in hj}
            return {t: pv(s, *t, ps[t]) for t in hj}
        def cat(oss, j0, j1):
            return jnp.concatenate([jnp.concatenate([os_[(h, j)] for j in range(j0, j1)], axis=0) for os_ in oss for h in range(G)], axis=1).astype(bf16)

        def group(s):
            return [(s, 1), (s, 2), (s, 3)] + ([(s + L, 0)] if s + L < NS else [])
        copy(0, 0).start()
        for c in xa_c: c.start()
        for s in range(1, L): copy(s, 0).start()
        for s in range(LA):
            for t in group(s): copy(*t).start()
        def dyn_copy(s, i, br):
            _, ks, vs, wqs, wos = srcs[br]
            g = s - br * NG
            c0 = pl.multiple_of(g * W, W)
            if i == 0: return pltpu.make_async_copy(wqs.at[:, pl.ds(c0, W)], wq_buf.at[s], sems.at[0, s])
            if i == 1: return pltpu.make_async_copy(ks.at[:, pl.ds(g * G, G)], k_buf.at[s], sems.at[1, s])
            if i == 2: return pltpu.make_async_copy(vs.at[:, pl.ds(g * G, G)], v_buf.at[s], sems.at[2, s])
            if i == 3: return pltpu.make_async_copy(wos.at[pl.ds(c0, W), :], wo_buf.at[s], sems.at[3, s])
        def dyn_start(s, ids):
            @pl.when(s < NG)
            def _():
                for i in ids: dyn_copy(s, i, 0).start()
            @pl.when(jnp.logical_and(s >= NG, s < NS))
            def _():
                for i in ids: dyn_copy(s, i, 1).start()
        acc[...] = jnp.zeros_like(acc)
        wait(0, 0)
        for c in range(XC):
            xa_c[c].wait()
            qproj(0, 0, c * RX, RX)
        for s in range(1, L):
            wait(s, 0)
            qproj(s, s)

        def step(s, carry):
            br = s // NG
            g = s - br * NG
            slot = s % L
            @pl.when(s == NG - L)
            def _():
                xb_c.wait()
            @pl.when(s == NG)
            def _():
                pltpu.make_async_copy(o_buf.at[0], out.at[:, pl.ds(0, D)], osem.at[0]).start()
            for i in (1, 2, 3): wait(s, i)
            wait(s + L, 0)
            dyn_start(s + LA, (1, 2, 3))
            dyn_start(s + LA + L, (0,))
            @pl.when(s == max(NG - L - 2, 0))
            def _():
                xb_c.start()
            o = cat([attn(s, slot)], 0, NQ)
            r = jnp.dot(o, wo_buf[s], preferred_element_type=f32)
            r = r + jnp.where(g > 0, acc[...], 0.0)
            acc[...] = r
            o_buf[br] = r.astype(bf16)
            qproj(s + L, slot)
            return carry
        jax.lax.fori_loop(0, NS - L, step, 0)

        last = range(NS - L, NS)
        for s in last:
            for i in (1, 2, 3): wait(s, i)
        oss = [attn(s, s % L) for s in last]
        wo = jnp.concatenate([wo_buf[s] for s in last], axis=0)
        cps = []
        r0 = 0
        for c, rc in enumerate(OC):
            rows = slice(r0, r0 + rc)
            o = cat(oss, r0 // 128, (r0 + rc) // 128)
            r = jnp.dot(o, wo, preferred_element_type=f32) + acc[rows]
            o_buf[1, rows] = r.astype(bf16)
            cp = pltpu.make_async_copy(o_buf.at[1, rows], out.at[rows, pl.ds(D, D)], osem.at[1 + c])
            cp.start()
            cps.append(cp)
            r0 += rc
        pltpu.make_async_copy(o_buf.at[0], out.at[:, pl.ds(0, D)], osem.at[0]).wait()
        for cp in cps: cp.wait()

    @jax.jit
    def f(A_x, A_k_cache, A_v_cache, A_wq, A_wo, B_x, B_k_cache, B_v_cache, B_wq, B_wo):
        out = pl.pallas_call(
            kern,
            in_specs=[pl.BlockSpec(memory_space=pl.ANY)] * 10,
            out_specs=pl.BlockSpec(memory_space=pl.ANY),
            out_shape=jax.ShapeDtypeStruct((M, 2 * D), bf16),
            scratch_shapes=[
                pltpu.VMEM((2, M, D), bf16),
                pltpu.VMEM((NS, B, G, SK, DH), bf16),
                pltpu.VMEM((NS, B, G, SK, DH), bf16),
                pltpu.VMEM((NS, D, W), bf16),
                pltpu.VMEM((NS, W, D), bf16),
                pltpu.VMEM((L, G, NQ, 64, 128), u32) if qT else pltpu.VMEM((L, M, W), bf16),
                pltpu.VMEM((M, D), f32),
                pltpu.VMEM((2, M, D), bf16),
                pltpu.SemaphoreType.DMA((5, NS)),
                pltpu.SemaphoreType.DMA((1 + XC,)),
                pltpu.SemaphoreType.DMA((1 + len(OC),)),
            ],
            compiler_params=pltpu.CompilerParams(vmem_limit_bytes=110 * 2**20, disable_bounds_checks=nobc),
            name="mha2",
        )(A_x.reshape(M, D), A_k_cache, A_v_cache, A_wq, A_wo, B_x.reshape(M, D), B_k_cache, B_v_cache, B_wq, B_wo)
        return out.reshape(B, SQ, 2 * D)
    return f


_impl = make(G=4)


@jax.jit
def pallas_concat_heads__mha_block_cached__mha_block_cached__near_ridge_kernel(
    A_x, A_k_cache, A_v_cache, A_wq, A_wo, B_x, B_k_cache, B_v_cache, B_wq, B_wo
):
    return _impl(A_x, A_k_cache, A_v_cache, A_wq, A_wo, B_x, B_k_cache, B_v_cache, B_wq, B_wo)
```

```python
import jax
import jax.numpy as jnp
import jax.experimental.pallas as pl
import jax.experimental.pallas.tpu as pltpu

B, SQ, D, H, SK, DH = 32, 32, 640, 32, 32, 128
M = B * SQ
NQ = B // 4
G = 4
NG = H // G
NS = 2 * NG
W = G * DH
LAG = 2
AHEAD = 2
XC = 4
RX = M // XC
OUT_CHUNKS = (512, 256, 128, 128)
SCORE_SCALE = DH ** -0.5 * 1.4426950408889634

F32, BF16, U32 = jnp.float32, jnp.bfloat16, jnp.uint32
WQ, K, V, WO = range(4)


def _kernel(xa, ka, va, wqa, woa, xb, kb, vb, wqb, wob, out,
            x_buf, k_buf, v_buf, wq_buf, wo_buf, q_buf, acc, o_buf, sems, osem):
    srcs = ((xa, ka, va, wqa, woa), (xb, kb, vb, wqb, wob))

    def copy(s, what, br):
        _, ks, vs, wqs, wos = srcs[br]
        g = s - br * NG
        c0 = g * W
        if not isinstance(c0, int):
            c0 = pl.multiple_of(c0, W)
        if what == WQ:
            src, dst = wqs.at[:, pl.ds(c0, W)], wq_buf
        elif what == K:
            src, dst = ks.at[:, pl.ds(g * G, G)], k_buf
        elif what == V:
            src, dst = vs.at[:, pl.ds(g * G, G)], v_buf
        else:
            src, dst = wos.at[pl.ds(c0, W), :], wo_buf
        return pltpu.make_async_copy(src, dst.at[s], sems.at[what, s])

    def start(s, whats):
        if isinstance(s, int):
            for what in whats:
                copy(s, what, s // NG).start()
            return

        @pl.when(s < NG)
        def _():
            for what in whats:
                copy(s, what, 0).start()

        @pl.when(jnp.logical_and(s >= NG, s < NS))
        def _():
            for what in whats:
                copy(s, what, 1).start()

    def wait(s, what):
        dst = (wq_buf, k_buf, v_buf, wo_buf)[what].at[s]
        pltpu.make_async_copy(dst, dst, sems.at[what, s]).wait()

    half = W // 2
    wq0_copies = [
        pltpu.make_async_copy(wqa.at[:, pl.ds(i * half, half)],
                              wq_buf.at[0, :, pl.ds(i * half, half)],
                              sems.at[4, 1 + XC + i])
        for i in range(2)]
    xa_copies = [
        pltpu.make_async_copy(xa.at[pl.ds(c * RX, RX)],
                              x_buf.at[0, pl.ds(c * RX, RX)], sems.at[4, 1 + c])
        for c in range(XC)]

    def xb_copy():
        return pltpu.make_async_copy(xb, x_buf.at[1], sems.at[4, 0])

    def out_a_copy():
        return pltpu.make_async_copy(o_buf.at[0], out.at[:, pl.ds(0, D)], osem.at[0])

    lane = jax.lax.broadcasted_iota(jnp.int32, (32, 128), 1)
    own = [lane // 32 == i for i in range(4)]

    def load_kv(buf, s, h, j):
        words = buf.bitcast(U32)[s, 4 * j:4 * j + 4, h].reshape(64, 128)
        return pltpu.bitcast(words, BF16)

    def q_proj(s, slot, r0=0, nr=M):
        q = jnp.dot(x_buf[s // NG, r0:r0 + nr], wq_buf[s], preferred_element_type=F32)
        q_buf[slot, r0:r0 + nr] = q.astype(BF16)

    def probs_t(s, slot, h, j):
        qt = q_buf[slot, j * 128:(j + 1) * 128, h * DH:(h + 1) * DH]
        kt = load_kv(k_buf, s, h, j)
        st = jax.lax.dot_general(kt, qt, (((1,), (1,)), ((), ())),
                                 preferred_element_type=F32)
        ct = jnp.where(own[0], st[0:32],
                       jnp.where(own[1], st[32:64],
                                 jnp.where(own[2], st[64:96], st[96:128])))
        m = jnp.max(ct, axis=0, keepdims=True)
        e = jnp.exp2((ct - m) * SCORE_SCALE)
        l = jnp.sum(e, axis=0, keepdims=True)
        return e * pl.reciprocal(l, approx=False)

    def p_times_v(s, h, j, pt):
        vt = load_kv(v_buf, s, h, j)
        pt_bd = jnp.concatenate([jnp.where(own[i], pt, 0.0) for i in range(4)],
                                axis=0).astype(BF16)
        return jax.lax.dot_general(pt_bd, vt, (((0,), (0,)), ((), ())),
                                   preferred_element_type=F32)

    def attention(s, slot):
        tiles = [(h, j) for h in range(G) for j in range(NQ)]
        pts = {t: probs_t(s, slot, *t) for t in tiles}
        return {t: p_times_v(s, *t, pts[t]) for t in tiles}

    def gather_o(os_list, j0, j1):
        cols = [jnp.concatenate([o[(h, j)] for j in range(j0, j1)], axis=0)
                for o in os_list for h in range(G)]
        return jnp.concatenate(cols, axis=1).astype(BF16)

    wq0_copies[0].start()
    xa_copies[0].start()
    wq0_copies[1].start()
    for cp in xa_copies[1:]:
        cp.start()
    for s in range(1, LAG):
        start(s, (WQ,))
    for s in range(AHEAD):
        start(s, (K, V, WO))
        if s + LAG < NS:
            start(s + LAG, (WQ,))

    acc[...] = jnp.zeros_like(acc)
    for c in range(XC):
        xa_copies[c].wait()
        if c == 0:
            for i in range(2):
                wq0_copies[i].wait()
                cols = slice(i * half, (i + 1) * half)
                q = jnp.dot(x_buf[0, 0:RX], wq_buf[0, :, cols],
                            preferred_element_type=F32)
                q_buf[0, 0:RX, cols] = q.astype(BF16)
        else:
            q_proj(0, 0, c * RX, RX)
    for s in range(1, LAG):
        wait(s, WQ)
        q_proj(s, s)

    def step(s, carry):
        br = s // NG
        g = s - br * NG
        slot = s % LAG

        @pl.when(s == NG - LAG)
        def _():
            xb_copy().wait()

        @pl.when(s == NG)
        def _():
            out_a_copy().start()

        for what in (K, V, WO):
            wait(s, what)
        wait(s + LAG, WQ)
        start(s + AHEAD, (K, V, WO))
        start(s + AHEAD + LAG, (WQ,))

        @pl.when(s == NG - LAG - 2)
        def _():
            xb_copy().start()

        o = gather_o([attention(s, slot)], 0, NQ)
        r = jnp.dot(o, wo_buf[s], preferred_element_type=F32)
        r = r + jnp.where(g > 0, acc[...], 0.0)
        acc[...] = r
        o_buf[br] = r.astype(BF16)
        q_proj(s + LAG, slot)
        return carry

    jax.lax.fori_loop(0, NS - LAG, step, 0)

    last = range(NS - LAG, NS)
    for s in last:
        for what in (K, V, WO):
            wait(s, what)
    os_list = [attention(s, s % LAG) for s in last]
    wo = jnp.concatenate([wo_buf[s] for s in last], axis=0)
    out_copies = []
    r0 = 0
    for c, rc in enumerate(OUT_CHUNKS):
        rows = slice(r0, r0 + rc)
        o = gather_o(os_list, r0 // 128, (r0 + rc) // 128)
        width = 128 if c == len(OUT_CHUNKS) - 1 else D
        for n in range(D // width):
            cols = slice(n * width, (n + 1) * width)
            r = jnp.dot(o, wo[:, cols], preferred_element_type=F32) + acc[rows, cols]
            o_buf[1, rows, cols] = r.astype(BF16)
            cp = pltpu.make_async_copy(
                o_buf.at[1, rows, cols],
                out.at[rows, pl.ds(D + n * width, width)],
                osem.at[1 + c + n])
            cp.start()
            out_copies.append(cp)
        r0 += rc
    out_a_copy().wait()
    for cp in out_copies:
        cp.wait()


@jax.jit
def pallas_concat_heads__mha_block_cached__mha_block_cached__near_ridge_kernel(
    A_x: jax.Array,
    A_k_cache: jax.Array,
    A_v_cache: jax.Array,
    A_wq: jax.Array,
    A_wo: jax.Array,
    B_x: jax.Array,
    B_k_cache: jax.Array,
    B_v_cache: jax.Array,
    B_wq: jax.Array,
    B_wo: jax.Array,
):
    out = pl.pallas_call(
        _kernel,
        in_specs=[pl.BlockSpec(memory_space=pl.ANY)] * 10,
        out_specs=pl.BlockSpec(memory_space=pl.ANY),
        out_shape=jax.ShapeDtypeStruct((M, 2 * D), BF16),
        scratch_shapes=[
            pltpu.VMEM((2, M, D), BF16),
            pltpu.VMEM((NS, B, G, SK, DH), BF16),
            pltpu.VMEM((NS, B, G, SK, DH), BF16),
            pltpu.VMEM((NS, D, W), BF16),
            pltpu.VMEM((NS, W, D), BF16),
            pltpu.VMEM((LAG, M, W), BF16),
            pltpu.VMEM((M, D), F32),
            pltpu.VMEM((2, M, D), BF16),
            pltpu.SemaphoreType.DMA((5, NS)),
            pltpu.SemaphoreType.DMA((len(OUT_CHUNKS) + D // 128,)),
        ],
        compiler_params=pltpu.CompilerParams(
            vmem_limit_bytes=110 * 2**20,
            disable_bounds_checks=True,
            flags={"XLA_TPU_RESCHEDULE_DMA_DONES": True},
        ),
        name="concat_heads_mha_cached",
    )(A_x.reshape(M, D), A_k_cache, A_v_cache, A_wq, A_wo,
      B_x.reshape(M, D), B_k_cache, B_v_cache, B_wq, B_wo)
    return out.reshape(B, SQ, 2 * D)
```
